```python
import os as _os
_os.environ.setdefault("JAX_PLATFORMS", "cpu")
import jax
import jax.numpy as jnp

def _softmax(x, axis=-1):
    return jax.nn.softmax(x, axis=axis)
def _gelu(x):
    return jax.nn.gelu(x, approximate=True)
def _silu(x):
    return jax.nn.silu(x)
def _sigmoid(x):
    return jax.nn.sigmoid(x)
def _layernorm(x, axis=-1, eps=1e-5):
    m = jnp.mean(x, axis=axis, keepdims=True)
    v = jnp.var(x, axis=axis, keepdims=True)
    return (x - m) / jnp.sqrt(v + eps)
def _scatter_add(tgt, idx, src, axis=0):
    return tgt.at[idx].add(src)
def _segment_sum(src, seg, n):
    return jax.ops.segment_sum(src, seg, n)
class _Rng:
    def __init__(self, key):
        self._k = key
    def _next(self):
        self._k, sub = jax.random.split(self._k)
        return sub
    def normal(self, shape):
        return jax.random.normal(self._next(), shape, dtype=jnp.bfloat16)
    def randint(self, lo, hi, shape):
        return jax.random.randint(self._next(), shape, lo, hi, dtype=jnp.int32)
    def uniform(self, shape, lo=0.0, hi=1.0):
        return jax.random.uniform(self._next(), shape, jnp.bfloat16, lo, hi)
    def permutation(self, n):
        return jax.random.permutation(self._next(), n)


kernel_name = 'interleave_layers__sliding_local_dilated__linear_kernel_hedgehog__prompt'

def setup_inputs():
    _rng = _Rng(jax.random.key(int.from_bytes(__import__("os").urandom(4), "little")))
    _w = (lambda a: (lambda t: t.astype(jnp.bfloat16) if jnp.issubdtype(t.dtype, jnp.floating) else t)(jnp.asarray(a)))
    def _A_setup():
        B, S, D = 1, 2048, 640
        return {
            "x": _w((lambda *s: _rng.normal(s) * 0.05)(B, S, D)),
            "wqkv": _w((lambda *s: _rng.normal(s) * 0.05)(D, 3 * D)),
            "wo": _w((lambda *s: _rng.normal(s) * 0.05)(D, D)),
        }
    _A_in = _A_setup()

    def _B_setup():
        B, S, D, H = 1, 2048, 640, 32
        Dh = D // H
        return {
            "x": _w((lambda *s: _rng.normal(s) * 0.05)(B, S, D)),
            "wqkv": _w((lambda *s: _rng.normal(s) * 0.4)(D, 3 * D)),
            "w_phi": _w((lambda *s: _rng.normal(s) * 0.4)(H, Dh, Dh) * (Dh ** -0.5)),
            "wo": _w((lambda *s: _rng.normal(s) * 0.1)(D, D)),
        }
    _B_in = _B_setup()

    return {
        "A_x": _A_in["x"],
        "A_wqkv": _A_in["wqkv"],
        "A_wo": _A_in["wo"],
        "B_x": _B_in["x"],
        "B_wqkv": _B_in["wqkv"],
        "B_w_phi": _B_in["w_phi"],
        "B_wo": _B_in["wo"],
    }

def reference(A_x, A_wqkv, A_wo, B_x, B_wqkv, B_w_phi, B_wo):
    def _A_ref(x, wqkv, wo):
        B, S, D = x.shape
        H = 32; Dh = D // H
        W, dil = 8, 2
        qkv = (lambda x, *d: x.transpose(*d))((x @ wqkv).reshape(B, S, 3, H, Dh), 2, 0, 3, 1, 4)
        q, k, v = qkv[0], qkv[1], qkv[2]
        scale = Dh ** -0.5
        pos = jnp.arange(S)
        off = jnp.arange(W) * dil
        idx = pos[:, None] - off[None, :]
        mask = idx >= 0
        idx_c = jnp.where(mask, idx, 0).reshape(-1)
        kg = k[:, :, idx_c, :].reshape(B, H, S, W, Dh)
        vg = v[:, :, idx_c, :].reshape(B, H, S, W, Dh)
        logits = jnp.einsum("bhsd,bhswd->bhsw", q, kg) * scale
        logits = jnp.where(mask[None, None, :, :], logits, -1e9)
        attn = _softmax(logits, axis=-1)
        o = jnp.einsum("bhsw,bhswd->bhsd", attn, vg)
        return (lambda x, *d: x.transpose(*d))(o, 0, 2, 1, 3).reshape(B, S, D) @ wo

    def _B_ref(x, wqkv, w_phi, wo):
        B, S, D = x.shape
        H = 32; Dh = D // H
        qkv = (lambda x, *d: x.transpose(*d))((x @ wqkv).reshape(B, S, 3, H, Dh), 2, 0, 3, 1, 4)
        q, k, v = qkv[0], qkv[1], qkv[2]
        pq = jnp.einsum("bhsd,hdf->bhsf", q, w_phi)
        pk = jnp.einsum("bhsd,hdf->bhsf", k, w_phi)
        phi_q = jnp.concatenate([_softmax(pq, axis=-1), _softmax(-pq, axis=-1)], axis=-1)
        phi_k = jnp.concatenate([_softmax(pk, axis=-1), _softmax(-pk, axis=-1)], axis=-1)
        kv = jnp.einsum("bhsf,bhsd->bhfd", phi_k, v)
        z  = jnp.einsum("bhsf->bhf", phi_k)
        num = jnp.einsum("bhqf,bhfd->bhqd", phi_q, kv)
        den = jnp.einsum("bhqf,bhf->bhq", phi_q, z)[..., None] + 1e-6
        o = num / den
        return (lambda x, *d: x.transpose(*d))(o, 0, 2, 1, 3).reshape(B, S, D) @ wo

    x = A_x
    x = x + _A_ref(_layernorm(x, axis=-1), A_wqkv, A_wo)
    x = x + _B_ref(_layernorm(x, axis=-1), B_wqkv, B_w_phi, B_wo)
    x = x + _A_ref(_layernorm(x, axis=-1), A_wqkv, A_wo)
    x = x + _B_ref(_layernorm(x, axis=-1), B_wqkv, B_w_phi, B_wo)
    return x
```

```python
import math

import jax
import jax.numpy as jnp
import jax.experimental.pallas as pl
import jax.experimental.pallas.tpu as pltpu

S = 2048
D = 640
H = 32
DH = 20
W = 8
G = 4
GR = 160
NJ = 8
HS = 1024
LOG2E = 1.4426950408889634
F32 = jnp.float32
BF16 = jnp.bfloat16


def _dot(a, b):
    return jnp.dot(a, b, preferred_element_type=F32)


def _dot_nt(a, b):
    return jax.lax.dot_general(a, b, (((1,), (1,)), ((), ())), preferred_element_type=F32)


def _tree(op, xs):
    xs = list(xs)
    while len(xs) > 1:
        nxt = [op(xs[i], xs[i + 1]) for i in range(0, len(xs) - 1, 2)]
        if len(xs) % 2:
            nxt.append(xs[-1])
        xs = nxt
    return xs[0]


def _chain(op, xs):
    acc = xs[0]
    for x in xs[1:]:
        acc = op(acc, x)
    return acc


MC = 160
NC = 8
JB = 1
MODE = 0


def _mix(mm, gen, n):
    k = len(mm)
    done = 0
    for i, f in enumerate(mm):
        if MODE != 1:
            f()
        if gen is not None:
            tgt = (i + 1) * n // k
            while done < tgt:
                next(gen, None)
                done += 1
        if MODE == 1:
            f()
    if gen is not None:
        for _ in gen:
            pass


UNR = ""


def loop(body, t):
    if t in UNR:
        for g in range(G - 1):
            body(g, None)
    else:
        jax.lax.fori_loop(0, G - 1, body, None)


def _rows(d):
    return slice(8 * d, 8 * d + 8)


def _cols(j):
    return slice(128 * j, 128 * j + 128)


def _kernel(x_hbm, aw_hbm, awo_hbm, bw_hbm, phi_hbm, bwo_hbm, out_hbm,
            xs, wraw_a, wraw_b, wo_raw_a, wo_raw_b, phi_raw,
            wa, wb, woa, wob, xt0, xt1, ht0, ht1, ot0, ot1,
            qkv0, qkv1, ext0, ext1, phq0, phq1, pq0, pq1, phk0, phk1,
            kvacc, kvm, lg, sem):
    xt = (xt0, xt1)
    ht = (ht0, ht1)
    ot = (ot0, ot1)
    qkv = (qkv0, qkv1)
    ext = (ext0, ext1)
    phq = (phq0, phq1)
    pqs = (pq0, pq1)
    phk = (phk0, phk1)

    x_cp = [pltpu.make_async_copy(x_hbm.at[:, _cols(c)], xs.at[c], sem.at[c]) for c in range(5)]
    a_cp = [pltpu.make_async_copy(aw_hbm.at[:, D * m:D * m + D], wraw_a.at[:, D * m:D * m + D], sem.at[5 + m])
            for m in range(3)]
    w_cp = [pltpu.make_async_copy(s, d, sem.at[8 + i]) for i, (s, d) in enumerate(
        [(awo_hbm, wo_raw_a), (bw_hbm, wraw_b), (phi_hbm, phi_raw), (bwo_hbm, wo_raw_b)])]
    for c in x_cp + a_cp:
        c.start()

    xs32 = xs.bitcast(jnp.uint32)
    for c in range(5):
        x_cp[c].wait()
        if c == 2:
            for cp in w_cp:
                cp.start()
        for j in range(NJ):
            blk = xs32[c, pl.ds(j, 128, stride=8), :].T
            xt0[_cols(c), _cols(j)] = pltpu.bitcast(blk << 16, F32)
            xt1[_cols(c), _cols(j)] = pltpu.bitcast(blk & jnp.uint32(0xFFFF0000), F32)

    r_i = jax.lax.broadcasted_iota(jnp.int32, (GR, 256), 0)
    c_i = jax.lax.broadcasted_iota(jnp.int32, (GR, 256), 1)
    r_h = r_i & 7
    r_d = r_i >> 3

    r_q = r_i >= 80
    b_h = (r_i & 3) + jnp.where(r_q, 4, 0)
    b_d = (jnp.where(r_q, r_i - 80, r_i) >> 3) * 2 + ((r_i >> 2) & 1)

    def perm(g, b=False):
        tgt = 32 * g + (20 * b_h + b_d if b else 20 * r_h + r_d)
        return jnp.where(c_i == tgt, 1.0, 0.0).astype(BF16)

    def prep_w(raw, dst, m, g, mat, scale=None):
        v = _dot_nt(mat, raw[:, 640 * m + 128 * g: 640 * m + 128 * g + 256])
        if scale is not None:
            v = v * scale
        dst[g, GR * m: GR * m + GR, :] = v.astype(BF16)

    def prep_wo(raw, dst, b, tmp):
        for g in range(G):
            tmp[GR * g: GR * g + GR, 0:640] = _dot(perm(g, b), raw[128 * g: 128 * g + 256, :])
        dst[...] = tmp[0:640, 0:640].T.astype(BF16)

    pms = [perm(g) for g in range(G)]
    for m in range(3):
        a_cp[m].wait()
        for g in range(G):
            prep_w(wraw_a, wa, m, g, pms[g])

    def prep_rest():
        for cp in w_cp:
            cp.wait()
        prep_wo(wo_raw_a, woa, False, pq0)
        prep_wo(wo_raw_b, wob, True, pq1)
        erep = jnp.where(b_d[:, :DH] == c_i[:, :DH], 1.0, 0.0).astype(BF16)
        for g in range(G):
            t = _dot_nt(erep, phi_raw[128 * g: 128 * g + 256, :])
            lo = 32 * g + 20 * b_h
            mg = jnp.where((c_i >= lo) & (c_i < lo + 20), t, 0.0).astype(BF16)
            prep_w(wraw_b, wb, 0, g, mg, LOG2E)
            prep_w(wraw_b, wb, 1, g, mg, LOG2E)
            prep_w(wraw_b, wb, 2, g, perm(g, True))

    lane0 = jax.lax.broadcasted_iota(jnp.int32, (8, 128), 1) == 0

    def ln(p):
        for j in range(NJ):
            x = xt[p][:, _cols(j)]
            m = jnp.sum(x, axis=0, keepdims=True) * (1.0 / D)
            xc = x - m
            v = jnp.sum(xc * xc, axis=0, keepdims=True) * (1.0 / D)
            ht[p][:, _cols(j)] = (xc * jax.lax.rsqrt(v + 1e-5)).astype(BF16)

    def proj_a(g, p):
        def mk(r0, r1, j0, j1):
            def f():
                r = _dot(wa[g, r0:r1, :], ht[p][:, 128 * j0:128 * j1])
                qkv[p][r0:r1, 128 * j0:128 * j1] = r
                lo = max(r0, GR)
                if lo < r1:
                    for j in range(max(j0, 1), j1):
                        ext[p][lo - GR:r1 - GR, _cols(j - 1)] = pltpu.roll(r[lo - r0:, _cols(j - j0)], 1, axis=1)
            return f
        return [mk(r0, r0 + MC, j0, j0 + NC) for r0 in range(0, 480, MC) for j0 in range(0, NJ, NC)]

    def kvext(p, m, d, e):
        if e >= 7:
            return qkv[p][pl.ds(GR * (m + 1) + 8 * d, 8), _cols(e - 7)]
        return ext[p][pl.ds(GR * m + 8 * d, 8), _cols(e)]

    def att(g, p, JB=4):
        cs = DH ** -0.5 * LOG2E
        row0 = g * GR if isinstance(g, int) else pl.multiple_of(g * GR, 32)
        for jb in range(0, NJ, JB):
            js = range(jb, jb + JB)
            acc = {}
            for d in range(DH):
                q = {j: qkv[p][_rows(d), _cols(j)] for j in js}
                for e in range(jb, jb + JB + 7):
                    k = kvext(p, 0, d, e)
                    for j in js:
                        w = j - e + 7
                        if 0 <= w < W:
                            t = q[j] * k
                            acc[j, w] = t if d == 0 else acc[j, w] + t
                yield
            for j in js:
                l = [acc[j, w] * cs for w in range(W)]
                l = [jnp.where(lane0, -1e9, l[w]) if j - w < 0 else l[w] for w in range(W)]
                mx = _tree(jnp.maximum, l)
                ex = [jnp.exp2(a - mx) for a in l]
                rs = 1.0 / _tree(jnp.add, ex)
                for w in range(W):
                    acc[j, w] = ex[w] * rs
                yield
            for d2 in range(0, DH, 2):
                o = {}
                for d in (d2, d2 + 1):
                    for e in range(jb, jb + JB + 7):
                        v = kvext(p, 1, d, e)
                        for j in js:
                            w = j - e + 7
                            if 0 <= w < W:
                                t = acc[j, w] * v
                                o[j, d] = o[j, d] + t if (j, d) in o else t
                    if d == d2:
                        yield
                for j in js:
                    ot[p][pl.ds(row0 + 8 * d2, 16), _cols(j)] = jnp.concatenate(
                        [o[j, d2], o[j, d2 + 1]], axis=0).astype(BF16)
                yield

    def oproj(wo, p):
        xt[p][...] += _dot(wo[...], ot[p][...])

    def layer_a(first):
        _mix(proj_a(0, 0), None, 0)
        ln(1)

        def body(g, _):
            _mix(proj_a(g, 1), att(g, 0, JB), 88)
            _mix(proj_a(g + 1, 0), att(g, 1, JB), 88)
        loop(body, 'A')
        if first:
            prep_rest()
        _mix(proj_a(G - 1, 1), att(G - 1, 0, JB), 88)
        _mix([lambda: oproj(woa, 0)], att(G - 1, 1, JB), 88)
        oproj(woa, 1)
        ln(0)

    def swap4(a):
        return pltpu.roll(a, 4, axis=0)

    def dual_softmax(load, dst, r0, j):
        x = [load(f) for f in range(10)]
        mx = _tree(jnp.maximum, x)
        mn = _tree(jnp.minimum, x)
        mx = jnp.maximum(mx, swap4(mx))
        mn = jnp.minimum(mn, swap4(mn))
        for s in range(2):
            ex = [jnp.exp2(a - mx) if s == 0 else jnp.exp2(mn - a) for a in x]
            sm = _tree(jnp.add, ex)
            rs = 1.0 / (sm + swap4(sm))
            for f in range(0, 10, 2):
                r = r0 + 80 * s + 8 * f
                dst[r:r + 16, _cols(j)] = jnp.concatenate([ex[f] * rs, ex[f + 1] * rs], axis=0).astype(BF16)

    kv_ok = (jax.lax.broadcasted_iota(jnp.int32, (96, GR), 0) & 3) == (
        jax.lax.broadcasted_iota(jnp.int32, (96, GR), 1) & 3)

    def proj_kv(g, p):
        qkv[p][0:320, :] = _dot(wb[g, GR:, :], ht[p][...])

    def skv(g, p):
        for q in range(2):
            for j in range(NJ):
                dual_softmax(lambda f: qkv[p][_rows(10 * q + f), _cols(j)], phk[p], GR * q, j)
            va = jnp.concatenate([qkv[p][GR + 80 * q:GR + 80 * q + 80, :], jnp.ones((16, HS), F32)],
                                 axis=0).astype(BF16)
            r = _dot_nt(va, phk[p][GR * q:GR * q + GR, :])
            if p == 0:
                kvacc[q] = r
            else:
                kvm[2 * g + q, :, 0:GR] = jnp.where(kv_ok, kvacc[q] + r, 0.0).astype(BF16)

    def proj_q(p):
        pqs[p][...] = _dot(wb[:, 0:GR, :].reshape(D, D), ht[p][...])

    def smq(p):
        for q in range(2 * G):
            for j in range(NJ):
                dual_softmax(lambda f: pqs[p][_rows(10 * q + f), _cols(j)], phq[p], GR * q, j)

    def num(p):
        for q in range(2 * G):
            n = _dot(kvm[q, :, 0:GR], phq[p][GR * q:GR * q + GR, :])
            rs = 1.0 / (n[80:88, :] + 1e-6)
            for d in range(0, 10, 2):
                ot[p][80 * q + 8 * d: 80 * q + 8 * d + 16, :] = jnp.concatenate(
                    [n[_rows(d), :] * rs, n[_rows(d + 1), :] * rs], axis=0).astype(BF16)

    o_cp = [pltpu.make_async_copy(xs.at[c], out_hbm.at[:, _cols(c)], sem.at[c]) for c in range(5)]

    def layer_b(last):
        proj_kv(0, 0)
        ln(1)

        def body(g, _):
            proj_kv(g, 1)
            skv(g, 0)
            proj_kv(g + 1, 0)
            skv(g, 1)
        loop(body, 'B')
        proj_kv(G - 1, 1)
        skv(G - 1, 0)
        proj_q(0)
        skv(G - 1, 1)
        proj_q(1)
        smq(0)
        num(0)
        oproj(wob, 0)
        smq(1)
        num(1)
        if not last:
            oproj(wob, 1)
            ln(0)
            return
        for c in range(5):
            x1 = xt1[_cols(c), :] + _dot(wob[_cols(c), :], ot1[...])
            for j in range(NJ):
                pk = (pltpu.bitcast(xt0[_cols(c), _cols(j)].astype(BF16).astype(F32), jnp.uint32) >> 16) | pltpu.bitcast(
                    x1[:, _cols(j)].astype(BF16).astype(F32), jnp.uint32)
                xs32[c, pl.ds(j, 128, stride=8), :] = pk.astype(jnp.uint32).T
            o_cp[c].start()

    ln(0)
    for it in range(2):
        layer_a(it == 0)
        layer_b(it == 1)
    for c in o_cp:
        c.wait()


def _scratch():
    V = pltpu.VMEM
    return [
        V((5, S, 128), BF16),
        V((D, 3 * D), BF16), V((D, 3 * D), BF16),
        V((D, D), BF16), V((D, D), BF16), V((D, DH), BF16),
        V((G, 3 * GR, D), BF16), V((G, 3 * GR, D), BF16),
        V((D, D), BF16), V((D, D), BF16),
        V((D, HS), F32), V((D, HS), F32),
        V((D, HS), BF16), V((D, HS), BF16),
        V((D, HS), BF16), V((D, HS), BF16),
        V((480, HS), F32), V((480, HS), F32),
        V((2 * GR, 7 * 128), F32), V((2 * GR, 7 * 128), F32),
        V((2 * D, HS), BF16), V((2 * D, HS), BF16),
        V((D, HS), F32), V((D, HS), F32),
        V((2 * GR, HS), BF16), V((2 * GR, HS), BF16),
        V((2, 96, GR), F32), V((2 * G, 96, GR), BF16),
        V((256, 128), F32),
        pltpu.SemaphoreType.DMA((12,)),
    ]


@jax.jit
def pallas_interleave_layers__sliding_local_dilated__linear_kernel_hedgehog__prompt_kernel(
    A_x: jax.Array,
    A_wqkv: jax.Array,
    A_wo: jax.Array,
    B_x: jax.Array,
    B_wqkv: jax.Array,
    B_w_phi: jax.Array,
    B_wo: jax.Array,
):
    del B_x
    any_spec = pl.BlockSpec(memory_space=pltpu.HBM)
    out = pl.pallas_call(
        _kernel,
        out_shape=jax.ShapeDtypeStruct((S, D), BF16),
        in_specs=[any_spec] * 6,
        out_specs=any_spec,
        scratch_shapes=_scratch(),
        compiler_params=pltpu.CompilerParams(vmem_limit_bytes=100 * 1024 * 1024),
    )(A_x.reshape(S, D), A_wqkv, A_wo, B_wqkv, B_w_phi.reshape(D, DH), B_wo)
    return out.reshape(1, S, D)
```
